```python
import jax
import jax.numpy as jnp

def _softmax(x, axis=-1):
    return jax.nn.softmax(x, axis=axis)
def _gelu(x):
    return jax.nn.gelu(x, approximate=True)
def _silu(x):
    return jax.nn.silu(x)
def _sigmoid(x):
    return jax.nn.sigmoid(x)
def _layernorm(x, axis=-1, eps=1e-5):
    m = jnp.mean(x, axis=axis, keepdims=True)
    v = jnp.var(x, axis=axis, keepdims=True)
    return (x - m) / jnp.sqrt(v + eps)
def _scatter_add(tgt, idx, src, axis=0):
    return tgt.at[idx].add(src)
def _segment_sum(src, seg, n):
    return jax.ops.segment_sum(src, seg, n)
class _Rng:
    def __init__(self, key):
        self._k = key
    def _next(self):
        self._k, sub = jax.random.split(self._k)
        return sub
    def normal(self, shape):
        return jax.random.normal(self._next(), shape, dtype=jnp.bfloat16)
    def randint(self, lo, hi, shape):
        return jax.random.randint(self._next(), shape, lo, hi, dtype=jnp.int32)
    def uniform(self, shape, lo=0.0, hi=1.0):
        return jax.random.uniform(self._next(), shape, jnp.bfloat16, lo, hi)
    def permutation(self, n):
        return jax.random.permutation(self._next(), n)


kernel_name = 'recurrent_scan__sliding_local_dilated__swiglu_ffn__prompt'

def setup_inputs():
    _rng = _Rng(jax.random.key(int.from_bytes(__import__("os").urandom(4), "little")))
    _w = (lambda a: (lambda t: t.astype(jnp.bfloat16) if jnp.issubdtype(t.dtype, jnp.floating) else t)(jnp.asarray(a)))
    def _A_setup():
        B, S, D = 1, 2048, 1024
        return {
            "x": _w((lambda *s: _rng.normal(s) * 0.05)(B, S, D)),
            "wqkv": _w((lambda *s: _rng.normal(s) * 0.05)(D, 3 * D)),
            "wo": _w((lambda *s: _rng.normal(s) * 0.05)(D, D)),
        }
    _A_in = _A_setup()

    def _B_setup():
        B, S, D, F = 1, 2048, 1024, 3584
        return {
            "x": _w((lambda *s: _rng.normal(s) * 0.05)(B, S, D)),
            "w_gate": _w((lambda *s: _rng.normal(s) * 0.05)(D, F)),
            "w_up": _w((lambda *s: _rng.normal(s) * 0.05)(D, F)),
            "w_down": _w((lambda *s: _rng.normal(s) * 0.05)(F, D)),
        }
    _B_in = _B_setup()

    return {
        "A_x": _A_in["x"],
        "A_wqkv": _A_in["wqkv"],
        "A_wo": _A_in["wo"],
        "B_x": _B_in["x"],
        "B_w_gate": _B_in["w_gate"],
        "B_w_up": _B_in["w_up"],
        "B_w_down": _B_in["w_down"],
    }

def reference(A_x, A_wqkv, A_wo, B_x, B_w_gate, B_w_up, B_w_down):
    def _A_ref(x, wqkv, wo):
        B, S, D = x.shape
        H = 32; Dh = D // H
        W, dil = 8, 2
        qkv = (lambda x, *d: x.transpose(*d))((x @ wqkv).reshape(B, S, 3, H, Dh), 2, 0, 3, 1, 4)
        q, k, v = qkv[0], qkv[1], qkv[2]
        scale = Dh ** -0.5
        pos = jnp.arange(S)
        off = jnp.arange(W) * dil
        idx = pos[:, None] - off[None, :]
        mask = idx >= 0
        idx_c = jnp.where(mask, idx, 0).reshape(-1)
        kg = k[:, :, idx_c, :].reshape(B, H, S, W, Dh)
        vg = v[:, :, idx_c, :].reshape(B, H, S, W, Dh)
        logits = jnp.einsum("bhsd,bhswd->bhsw", q, kg) * scale
        logits = jnp.where(mask[None, None, :, :], logits, -1e9)
        attn = _softmax(logits, axis=-1)
        o = jnp.einsum("bhsw,bhswd->bhsd", attn, vg)
        return (lambda x, *d: x.transpose(*d))(o, 0, 2, 1, 3).reshape(B, S, D) @ wo

    def _B_ref(x, w_gate, w_up, w_down):
        g = _silu(x @ w_gate)
        u = x @ w_up
        return (g * u) @ w_down

    x = A_x
    xn = _layernorm(x, axis=-1)
    s = _A_ref(xn, A_wqkv, A_wo)
    g = _silu(_B_ref(xn, B_w_gate, B_w_up, B_w_down))
    return x + s * g
```

```python
import functools
import numpy as np
import jax, jax.numpy as jnp
from jax import lax
import jax.experimental.pallas as pl
import jax.experimental.pallas.tpu as pltpu

S, D, F, H, DH = 2048, 1024, 3584, 32, 32
W, DIL = 8, 2
HALO = 16
f32, bf16 = jnp.float32, jnp.bfloat16

def _dot(a, b):
    return jnp.dot(a, b, preferred_element_type=f32)

def _sigmoid(x):
    return 0.5 * jnp.tanh(0.5 * x) + 0.5

def _kernel(x_ref, wqkv_ref, wo_ref, wg_ref, wu_ref, wd_ref, o_ref, k_scr, v_scr, *, M, FC):
    i = pl.program_id(0)

    @pl.when(i == 0)
    def _():
        k_scr[0:HALO, :] = jnp.zeros((HALO, D), f32)
        v_scr[0:HALO, :] = jnp.zeros((HALO, D), f32)

    x = x_ref[...].astype(f32)
    mu = jnp.mean(x, axis=-1, keepdims=True)
    xc = x - mu
    var = jnp.mean(xc * xc, axis=-1, keepdims=True)
    xn = (xc * lax.rsqrt(var + 1e-5)).astype(bf16)

    q = _dot(xn, wqkv_ref[:, 0:D]) * (DH ** -0.5)
    k_scr[HALO:HALO + M, :] = _dot(xn, wqkv_ref[:, D:2 * D])
    v_scr[HALO:HALO + M, :] = _dot(xn, wqkv_ref[:, 2 * D:3 * D])

    r_i = lax.broadcasted_iota(jnp.int32, (128, 128), 0) // DH
    c_i = lax.broadcasted_iota(jnp.int32, (128, 128), 1) // DH
    E = jnp.where(r_i == c_i, 1.0, 0.0).astype(bf16)
    rows = i * M + lax.broadcasted_iota(jnp.int32, (M, 128), 0)
    outs = []
    for c in range(D // 128):
        cs = slice(c * 128, (c + 1) * 128)
        qc = q[:, cs]
        ls = []
        for w in range(W):
            ks = k_scr[HALO - DIL * w:HALO - DIL * w + M, cs]
            l = _dot((qc * ks).astype(bf16), E)
            if w > 0:
                l = jnp.where(rows >= DIL * w, l, -1e9)
            ls.append(l)
        m = functools.reduce(jnp.maximum, ls)
        ps = [jnp.exp(l - m) for l in ls]
        den = functools.reduce(jnp.add, ps)
        acc = None
        for w in range(W):
            vs = v_scr[HALO - DIL * w:HALO - DIL * w + M, cs]
            t = ps[w] * vs
            acc = t if acc is None else acc + t
        outs.append((acc / den).astype(bf16))
    o = jnp.concatenate(outs, axis=1)
    s = _dot(o, wo_ref[...])

    k_scr[0:HALO, :] = k_scr[M:M + HALO, :]
    v_scr[0:HALO, :] = v_scr[M:M + HALO, :]

    acc = None
    for c in range(F // FC):
        fs = slice(c * FC, (c + 1) * FC)
        g = _dot(xn, wg_ref[:, fs])
        u = _dot(xn, wu_ref[:, fs])
        h = (g * _sigmoid(g) * u).astype(bf16)
        t = _dot(h, wd_ref[fs, :])
        acc = t if acc is None else acc + t
    gate = acc * _sigmoid(acc)
    o_ref[...] = (x + s * gate).astype(bf16)


@jax.jit
def pallas_recurrent_scan__sliding_local_dilated__swiglu_ffn__prompt_kernel(A_x, A_wqkv, A_wo, B_x, B_w_gate, B_w_up, B_w_down):
    M, FC = 256, 512
    x2 = A_x.reshape(S, D)
    full = lambda shape: pl.BlockSpec(shape, lambda i: (0, 0), pipeline_mode=pl.Buffered(1))
    out = pl.pallas_call(
        functools.partial(_kernel, M=M, FC=FC),
        grid=(S // M,),
        in_specs=[pl.BlockSpec((M, D), lambda i: (i, 0)), full((D, 3 * D)), full((D, D)), full((D, F)), full((D, F)), full((F, D))],
        out_specs=pl.BlockSpec((M, D), lambda i: (i, 0)),
        out_shape=jax.ShapeDtypeStruct((S, D), bf16),
        scratch_shapes=[pltpu.VMEM((M + HALO, D), f32), pltpu.VMEM((M + HALO, D), f32)],
        compiler_params=pltpu.CompilerParams(dimension_semantics=("arbitrary",), vmem_limit_bytes=120 * 1024 * 1024),
    )(x2, A_wqkv, A_wo, B_w_gate, B_w_up, B_w_down)
    return out.reshape(1, S, D)
```

```python
import functools
import numpy as np
import jax, jax.numpy as jnp
from jax import lax
import jax.experimental.pallas as pl
import jax.experimental.pallas.tpu as pltpu

S, D, F, H, DH = 2048, 1024, 3584, 32, 32
W, DIL = 8, 2
HALO = 16
LN = 128
f32, bf16, u32 = jnp.float32, jnp.bfloat16, jnp.uint32


def _dot(a, b):
    return jnp.dot(a, b, preferred_element_type=f32)


def _silu(x):
    hx = 0.5 * x
    return hx * jnp.tanh(hx) + hx


def _kernel(x_hbm, wqkv_hbm, wo_hbm, wg_hbm, wu_hbm, wd_hbm, o_hbm,
            x_v, wqkv_v, wo_v, wg_v, wu_v, wd_v, wp_v, wop_v, tscr, xn_v, qkv_v, o_v, acc_v, h_v, out_v,
            sems, osems, *, M, FC, T, INFLIGHT, ATT, PERM_AT, SPLIT0):
    NB = S // M
    NC = F // FC
    NT = FC // LN

    jobs = {}
    order = []

    def add(name, src, dst):
        jobs[name] = pltpu.make_async_copy(src, dst, sems.at[len(order)])
        order.append(name)

    def add_x(b):
        add(("x", b), x_hbm.at[pl.ds(b * M, M), :], x_v.at[pl.ds(b * M, M), :])

    def add_c(c):
        cs = pl.ds(c * FC, FC)
        add(("g", c), wg_hbm.at[:, cs], wg_v.at[:, cs])
        add(("u", c), wu_hbm.at[:, cs], wu_v.at[:, cs])
        add(("d", c), wd_hbm.at[cs, :], wd_v.at[cs, :])

    add_x(0)
    for c in range(NC):
        add_c(c)
        if c == PERM_AT - 1:
            for m in range(3):
                add(("qkv", m), wqkv_hbm.at[:, pl.ds(m * D, D)], wqkv_v.at[:, pl.ds(m * D, D)])
        if c == PERM_AT:
            add("wo", wo_hbm, wo_v)
    for b in range(1, NB):
        add_x(b)
    started = [0]
    waited = set()

    def start_upto(n):
        while started[0] < min(n, len(order)):
            jobs[order[started[0]]].start()
            started[0] += 1

    def wait(name):
        if name in waited:
            return
        idx = order.index(name)
        start_upto(idx + 1)
        jobs[name].wait()
        waited.add(name)
        start_upto(max(order.index(n) for n in waited) + 1 + INFLIGHT)

    start_upto(INFLIGHT + 1)

    def ln(b, r0, n):
        wait(("x", b))
        rs = pl.ds(b * M + r0, n)
        x = x_v[rs, :].astype(f32)
        mu = jnp.mean(x, axis=-1, keepdims=True)
        xc = x - mu
        var = jnp.mean(xc * xc, axis=-1, keepdims=True)
        xn_v[rs, :] = (xc * lax.rsqrt(var + 1e-5)).astype(bf16)

    def ln_tasks(b, n=64):
        return [functools.partial(ln, b, r0, n) for r0 in range(0, M, n)]

    def perm_w(m, kt):
        wait(("qkv", m))
        ts = tscr.at[(m * 4 + kt) % 2]
        ks = slice(kt * 256, (kt + 1) * 256)
        for a in range(8):
            t = pltpu.bitcast(wqkv_v[ks, m * D + a * LN: m * D + (a + 1) * LN], u32).T
            for hh in range(4):
                ts[pl.ds(97 * (4 * a + hh), 32, stride=3), :] = t[hh * 32:(hh + 1) * 32, :]
        for c in range(8):
            t = jnp.concatenate([ts[pl.ds(3 * (4 * c + dq), 32, stride=97), :] for dq in range(4)], axis=0)
            wp_v[ks, m * D + c * LN: m * D + (c + 1) * LN] = pltpu.bitcast(t.T, bf16)

    def perm_wo(c):
        wait("wo")
        ts = tscr.at[c % 2]
        cs = slice(c * LN, (c + 1) * LN)
        for h in range(H):
            ts[pl.ds(97 * h, 32, stride=3), :] = pltpu.bitcast(wo_v[h * 32:(h + 1) * 32, cs].astype(f32), u32)
        for d2 in range(DH // 2):
            t = jnp.concatenate([ts[pl.ds(3 * (2 * d2 + e), 32, stride=97), :] for e in range(2)], axis=0)
            wop_v[d2 * 64:(d2 + 1) * 64, cs] = pltpu.bitcast(t, f32).astype(bf16)

    def qrow(r):
        return 3 * (HALO + r)

    def qkv_tile(b, m, c):
        y = _dot(xn_v[b * M:(b + 1) * M, :], wp_v[:, m * D + c * LN: m * D + (c + 1) * LN])
        slot = (2, 0, 1)[m]
        if m == 0:
            y = y * (DH ** -0.5)
        qkv_v[c, pl.ds(qrow(b * M) + slot, M, stride=3), :] = y

    def att_tile(b, r0):
        n = 8 * T
        g0 = b * M + r0
        ls = [None] * W
        for c in range(8):
            q = qkv_v[c, pl.ds(qrow(g0) + 2, n, stride=3), :]
            for w in range(W):
                k = qkv_v[c, pl.ds(qrow(g0 - DIL * w), n, stride=3), :]
                ls[w] = q * k if c == 0 else ls[w] + q * k
        for w in range(W):
            l = ls[w]
            l = l + pltpu.roll(l, 64, 1)
            l = l + pltpu.roll(l, 32, 1)
            if g0 < DIL * w:
                rows = g0 + lax.broadcasted_iota(jnp.int32, (n, LN), 0)
                l = jnp.where(rows >= DIL * w, l, -1e9)
            ls[w] = l
        mx = functools.reduce(jnp.maximum, ls)
        ps = [jnp.exp(l - mx) for l in ls]
        r = 1.0 / functools.reduce(jnp.add, ps)
        ps = [p * r for p in ps]
        for c in range(8):
            acc = None
            for w in range(W):
                v = qkv_v[c, pl.ds(qrow(g0 - DIL * w) + 1, n, stride=3), :]
                acc = ps[w] * v if w == 0 else acc + ps[w] * v
            o_v[pl.ds(g0, n), c * LN:(c + 1) * LN] = acc.astype(bf16)

    def att_tasks(b):
        return [functools.partial(att_tile, b, r0) for r0 in range(0, M, 8 * T)]

    def gu_tile(b, c, j):
        wait(("g", c)); wait(("u", c))
        xn = xn_v[b * M:(b + 1) * M, :]
        fs = slice(c * FC + j * LN, c * FC + (j + 1) * LN)
        g = _dot(xn, wg_v[:, fs])
        u = _dot(xn, wu_v[:, fs])
        h_v[c % 2, :, j * LN:(j + 1) * LN] = (_silu(g) * u).astype(bf16)

    def down_tile(b, c, n):
        wait(("d", c))
        t = _dot(h_v[c % 2], wd_v[c * FC:(c + 1) * FC, n * LN:(n + 1) * LN])
        ns = slice(n * LN, (n + 1) * LN)
        if c == 0:
            acc_v[b % 2, :, ns] = t
        else:
            acc_v[b % 2, :, ns] = acc_v[b % 2, :, ns] + t

    def ffn_steps(b, c):
        return [functools.partial(gu_tile, b, c, j) for j in range(NT)] + \
               [functools.partial(down_tile, b, c, n) for n in range(D // LN)]

    out_jobs = []

    def wo_tile(b, n):
        ns = slice(n * LN, (n + 1) * LN)
        s = _dot(o_v[b * M:(b + 1) * M, :], wop_v[:, ns])
        gate = _silu(acc_v[b % 2, :, ns])
        x = x_v[b * M:(b + 1) * M, ns].astype(f32)
        out_v[b * M:(b + 1) * M, ns] = (x + s * gate).astype(bf16)

    def out_dma(b, n0, n1):
        cp = pltpu.make_async_copy(out_v.at[pl.ds(b * M, M), pl.ds(n0 * LN, (n1 - n0) * LN)],
                                   o_hbm.at[pl.ds(b * M, M), pl.ds(n0 * LN, (n1 - n0) * LN)], osems.at[len(out_jobs)])
        cp.start()
        out_jobs.append(cp)

    def interleave(main, side):
        ns, nm = len(side), len(main)
        done = 0
        for i, step in enumerate(main):
            step()
            upto = (ns * (i + 1) + nm - 1) // nm if nm else ns
            while done < min(upto, ns):
                side[done](); done += 1
        while done < ns:
            side[done](); done += 1

    zero = jnp.zeros((3 * HALO, LN), f32)
    for c in range(8):
        qkv_v[c, 0:3 * HALO, :] = zero
    for t in ln_tasks(0):
        t()
    perm_tasks = [functools.partial(perm_w, m, kt) for m in range(3) for kt in range(4)] + \
                 [functools.partial(perm_wo, c) for c in range(8)]
    for b in range(NB):
        if b == 0:
            pre = [s for c in range(SPLIT0) for s in ffn_steps(0, c)]
            npre = len(ffn_steps(0, 0)) * PERM_AT
            interleave(pre[:npre], [])
            interleave(pre[npre:], perm_tasks)
            rest = range(SPLIT0, NC)
        else:
            rest = range(NC)
        interleave([functools.partial(qkv_tile, b, m, c) for m in range(3) for c in range(8)], [])
        side = (att_tasks(b) if ATT else []) + (ln_tasks(b + 1) if b + 1 < NB else [])
        interleave([s for c in rest for s in ffn_steps(b, c)], side)
        for n in range(D // LN):
            wo_tile(b, n)
            if b + 1 < NB:
                if n == D // LN - 1:
                    out_dma(b, 0, D // LN)
            elif (n + 1) % 2 == 0:
                out_dma(b, n - 1, n + 1)
    for cp in out_jobs:
        cp.wait()
    for name in order:
        wait(name)


@jax.jit
def pallas_recurrent_scan__sliding_local_dilated__swiglu_ffn__prompt_kernel(A_x, A_wqkv, A_wo, B_x, B_w_gate, B_w_up, B_w_down):
    M = 512
    FC = 512
    T = 2
    INFLIGHT = 3
    ATT = 1
    PERM_AT = 2
    SPLIT0 = 4
    x2 = A_x.reshape(S, D)
    anyspec = pl.BlockSpec(memory_space=pl.ANY)
    nb = S // M
    out = pl.pallas_call(
        functools.partial(_kernel, M=M, FC=FC, T=T, INFLIGHT=INFLIGHT, ATT=ATT, PERM_AT=PERM_AT, SPLIT0=SPLIT0),
        in_specs=[anyspec] * 6,
        out_specs=anyspec,
        out_shape=jax.ShapeDtypeStruct((S, D), bf16),
        scratch_shapes=[
            pltpu.VMEM((S, D), bf16),
            pltpu.VMEM((D, 3 * D), bf16),
            pltpu.VMEM((D, D), bf16),
            pltpu.VMEM((D, F), bf16),
            pltpu.VMEM((D, F), bf16),
            pltpu.VMEM((F, D), bf16),
            pltpu.VMEM((D, 3 * D), bf16),
            pltpu.VMEM((D, D), bf16),
            pltpu.VMEM((2, 97 * 32, LN), u32),
            pltpu.VMEM((S, D), bf16),
            pltpu.VMEM((8, 3 * (S + HALO), LN), f32),
            pltpu.VMEM((S, D), bf16),
            pltpu.VMEM((2, M, D), f32),
            pltpu.VMEM((2, M, FC), bf16),
            pltpu.VMEM((S, D), bf16),
            pltpu.SemaphoreType.DMA((64,)),
            pltpu.SemaphoreType.DMA((16,)),
        ],
        compiler_params=pltpu.CompilerParams(vmem_limit_bytes=120 * 1024 * 1024),
    )(x2, A_wqkv, A_wo, B_w_gate, B_w_up, B_w_down)
    return out.reshape(1, S, D)
```

```python
import contextlib
import functools
import numpy as np
import jax, jax.numpy as jnp
from jax import lax
import jax.experimental.pallas as pl
import jax.experimental.pallas.tpu as pltpu

S, D, F, H, DH = 2048, 1024, 3584, 32, 32
W, DIL = 8, 2
HALO = 16
LN = 128
ND = D // LN
NF = F // LN
f32, bf16, u32 = jnp.float32, jnp.bfloat16, jnp.uint32


def _dot(a, b):
    return jnp.dot(a, b, preferred_element_type=f32)


def _silu(x):
    hx = 0.5 * x
    return hx * jnp.tanh(hx) + hx


def _kernel(x_hbm, wqkv_hbm, wo_hbm, wg_hbm, wu_hbm, wd_hbm, o_hbm,
            x_v, wqkv_v, wo_v, wg_v, wu_v, wd_v, wp_v, wop_v, tscr, xn_v, qkv_v, o_v, acc_v, h_v, out_v,
            zbuf, sems, osems, *, P):
    M, FC, T = P["M"], P["FC"], P["T"]
    NB, NC, NT = S // M, F // FC, FC // LN

    def scope(name):
        return jax.named_scope(name) if P["SCOPES"] else contextlib.nullcontext()

    wqkv16, wo16, wg16, wu16, wd16, out16 = (
        r.bitcast(bf16) for r in (wqkv_v, wo_v, wg_v, wu_v, wd_v, out_v))
    jobs, order = {}, []

    def add(name, pairs):
        sem = sems.at[len(order)]
        jobs[name] = [pltpu.make_async_copy(s_, d_, sem) for s_, d_ in pairs]
        order.append(name)

    def col(ref, t, rows=None):
        return ref.at[slice(None) if rows is None else rows, pl.ds(t * LN, LN)]

    def add_x(b, r0, n):
        rs = pl.ds(b * M + r0, n)
        add(("x", b, r0), [(x_hbm.at[rs, :], x_v.at[rs, :])])

    def add_gu(c, j0, j1):
        ts = range(c * NT + j0, c * NT + j1)
        add(("gu", c, j0), [(col(wg_hbm, t), wg16.at[t]) for t in ts] + [(col(wu_hbm, t), wu16.at[t]) for t in ts])

    def add_d(c):
        rs = pl.ds(c * FC, FC)
        add(("d", c), [(col(wd_hbm, t, rs), wd16.at[t, rs, :]) for t in range(ND)])

    def add_qkv(m):
        add(("qkv", m), [(col(wqkv_hbm, m * ND + t), wqkv16.at[m * ND + t]) for t in range(ND)])

    XP = P["XP"]
    ms = (2, 1, 0) if P["VFIRST"] else (0, 1, 2)
    if P["FENCE"]:
        add("z", [(x_hbm.at[pl.ds(0, 16), pl.ds(0, LN)], zbuf.bitcast(bf16).at[i]) for i in range(2)])
    for r0 in range(0, M, XP):
        add_x(0, r0, XP)
    G0 = [(0, 1), (1, 2), (2, 4)]
    for j0, j1 in G0:
        add_gu(0, j0, j1)
    add_d(0)
    for c in range(1, NC):
        add_gu(c, 0, NT)
        if c == 3:
            add_qkv(ms[2])
            add("wo", [(col(wo_hbm, t), wo16.at[t]) for t in range(ND)])
        if c == 2:
            add_qkv(ms[1])
        add_d(c)
        if c == 1:
            add_qkv(ms[0])
    for b in range(1, NB):
        add_x(b, 0, M)
    started, waited = [0], set()

    def start_upto(n):
        while started[0] < min(n, len(order)):
            for cp in jobs[order[started[0]]]:
                cp.start()
            started[0] += 1

    def inflight():
        return sum(len(jobs[n]) for n in order[:started[0]] if n not in waited)

    def refill():
        while started[0] < len(order) and inflight() + len(jobs[order[started[0]]]) <= P["QMAX"]:
            start_upto(started[0] + 1)

    def wait(*names):
        names = [n for n in names if n not in waited and n in jobs]
        if not names:
            return
        start_upto(max(order.index(n) for n in names) + 1)
        for n in names:
            for cp in jobs[n]:
                cp.wait()
            waited.add(n)
        refill()

    refill()
    WAIT_D = {c: [("d", c), ("gu", c + 1, 0)] for c in range(1, NC)}
    WAIT_D[0] = [("d", 0)]
    WAIT_D[1] += [("qkv", ms[0])]
    WAIT_D[2] += [("qkv", ms[1])]
    WAIT_D[3] += [("qkv", ms[2]), "wo"]
    WAIT_G = {1: [("gu", 1, 0)], 4: list(order)}

    if P["NOSTORE"]:
        wg_r, wu_r, wd_r, x_r = (pltpu.annotate(r, no_store=True) for r in (wg_v, wu_v, wd_v, x_v))
    else:
        wg_r, wu_r, wd_r, x_r = wg_v, wu_v, wd_v, x_v
    z = None
    if P["FENCE"]:
        wait("z")
        z = jnp.max(jnp.abs(pltpu.bitcast(zbuf[0] ^ zbuf[1], f32))).astype(jnp.int32)

    def fence(val):
        if P["FENCE"]:
            v = val[0:8, :]
            for i in range(1, val.shape[0] // 8):
                v = jnp.maximum(v, val[8 * i:8 * i + 8, :])
            qkv_v[7, pl.ds(pl.multiple_of(z + 3 * (S + HALO), 8), 8), :] = v

    def ld(ref, t, r0, n):
        return pltpu.bitcast(ref[t, pl.ds(r0 // 2, n // 2), :], bf16)

    def st(ref, t, r0, val):
        ref[t, pl.ds(r0 // 2, val.shape[0] // 2), :] = pltpu.bitcast(val, u32)

    def cat(ref, r0, n, nt=ND):
        return jnp.concatenate([ld(ref, t, r0, n) for t in range(nt)], axis=1)

    def ln(b, r0, n):
        if b == 0:
            wait(*[("x", 0, p0) for p0 in range((r0 // XP) * XP, r0 + n, XP)])
        g0 = b * M + r0
        x = x_r[pl.ds(g0, n), :].astype(f32)
        mu = jnp.mean(x, axis=-1, keepdims=True)
        xc = x - mu
        var = jnp.mean(xc * xc, axis=-1, keepdims=True)
        xn = (xc * lax.rsqrt(var + 1e-5)).astype(bf16)
        for t in range(ND):
            st(xn_v, t, g0, xn[:, t * LN:(t + 1) * LN])

    def ln_tasks(b):
        n = P["LNT"] if b > 0 else P["LNT0"]
        return [functools.partial(ln, b, r0, n) for r0 in range(0, M, n)]

    def perm_w(m, kt):
        ts = tscr.at[(m * 4 + kt) % 2]
        ks = slice(kt * 128, (kt + 1) * 128)
        for a in range(ND):
            t = wqkv_v[m * ND + a, ks, :].T
            for hh in range(4):
                ts[pl.ds(97 * (4 * a + hh), 32, stride=3), :] = t[hh * 32:(hh + 1) * 32, :]
        for c in range(ND):
            t = jnp.concatenate([ts[pl.ds(3 * (4 * c + dq), 32, stride=97), :] for dq in range(4)], axis=0)
            wp_v[m * ND + c, ks, :] = t.T

    def perm_wo(c):
        ts = tscr.at[c % 2]
        for h in range(H):
            ts[pl.ds(97 * h, 32, stride=3), :] = pltpu.bitcast(ld(wo_v, c, h * 32, 32).astype(f32), u32)
        for d2 in range(DH // 2):
            t = jnp.concatenate([ts[pl.ds(3 * (2 * d2 + e), 32, stride=97), :] for e in range(2)], axis=0)
            st(wop_v, c, d2 * 64, pltpu.bitcast(t, f32).astype(bf16))

    def qrow(r):
        return 3 * (HALO + r)

    def qkv_tile(b, m, c):
        y = _dot(cat(xn_v, b * M, M), ld(wp_v, m * ND + c, 0, D))
        if m == 0:
            y = y * (DH ** -0.5)
        qkv_v[c, pl.ds(qrow(b * M) + (2, 0, 1)[m], M, stride=3), :] = y

    def att_tile(b, r0):
        n = 8 * T
        g0 = b * M + r0
        ls = [None] * W
        if P["MODE"] == 0:
            for c in range(ND):
                q = qkv_v[c, pl.ds(qrow(g0) + 2, n, stride=3), :]
                for w in range(W):
                    k = qkv_v[c, pl.ds(qrow(g0 - DIL * w), n, stride=3), :]
                    ls[w] = q * k if c == 0 else ls[w] + q * k
        else:
            qs = [qkv_v[c, pl.ds(qrow(g0) + 2, n, stride=3), :] for c in range(ND)]
            for w in range(W):
                l = None
                for c in range(ND):
                    k = qkv_v[c, pl.ds(qrow(g0 - DIL * w), n, stride=3), :]
                    l = qs[c] * k if c == 0 else l + qs[c] * k
                fence(l)
                ls[w] = l
        for w in range(W):
            l = ls[w]
            if P["ROLL3"]:
                l = (l + pltpu.roll(l, 32, 1)) + (pltpu.roll(l, 64, 1) + pltpu.roll(l, 96, 1))
            else:
                l = l + pltpu.roll(l, 64, 1)
                l = l + pltpu.roll(l, 32, 1)
            if g0 < DIL * w:
                rows = g0 + lax.broadcasted_iota(jnp.int32, (n, LN), 0)
                l = jnp.where(rows >= DIL * w, l, -1e9)
            ls[w] = l
        mx = functools.reduce(jnp.maximum, ls)
        ps = [jnp.exp(l - mx) for l in ls]
        r = 1.0 / functools.reduce(jnp.add, ps)
        ps = [p * r for p in ps]
        fence(functools.reduce(jnp.maximum, ps))
        for c in range(ND):
            acc = None
            for w in range(W):
                v = qkv_v[c, pl.ds(qrow(g0 - DIL * w) + 1, n, stride=3), :]
                acc = ps[w] * v if w == 0 else acc + ps[w] * v
            fence(acc)
            if n >= 16:
                st(o_v, c, g0, acc.astype(bf16))
            else:
                raise NotImplementedError

    def att_tasks(b):
        return [functools.partial(att_tile, b, r0) for r0 in range(0, M, 8 * T)]

    def gu_tile(b, c, j):
        t = c * NT + j
        if b == 0 and c == 0:
            wait(*[("gu", 0, j0) for j0, j1 in G0 if j0 <= j < j1])
        if b == 0 and j == 0 and c in WAIT_G:
            wait(*WAIT_G[c])
        xn = cat(xn_v, b * M, M)
        g = _dot(xn, ld(wg_r, t, 0, D))
        u = _dot(xn, ld(wu_r, t, 0, D))
        st(h_v.at[c % 2], j, 0, (_silu(g) * u).astype(bf16))

    def down_tile(b, c, n):
        if b == 0 and n == 0:
            wait(*WAIT_D[c])
        t = _dot(cat(h_v.at[c % 2], 0, M, NT), ld(wd_r, n, c * FC, FC))
        if c == 0:
            acc_v[b % 2, n] = t
        else:
            acc_v[b % 2, n] = acc_v[b % 2, n] + t

    def ffn_steps(b, c):
        return [functools.partial(gu_tile, b, c, j) for j in range(NT)] + \
               [functools.partial(down_tile, b, c, n) for n in range(ND)]

    out_jobs = []

    def wo_tile(b, n):
        s = _dot(cat(o_v, b * M, M), ld(wop_v, n, 0, D))
        gate = _silu(acc_v[b % 2, n])
        st(out_v, n, b * M, (x_r[pl.ds(b * M, M), n * LN:(n + 1) * LN].astype(f32) + s * gate).astype(bf16))
        rs = pl.ds(b * M, M)
        cp = pltpu.make_async_copy(out16.at[n, rs, :], col(o_hbm, n, rs), osems.at[b * ND + n])
        cp.start()
        out_jobs.append(cp)

    def interleave(main, side):
        ns, nm, done = len(side), len(main), 0
        for i, step in enumerate(main):
            step()
            upto = (ns * (i + 1) + nm - 1) // nm
            while done < min(upto, ns):
                side[done]()
                done += 1
        while done < ns:
            side[done]()
            done += 1

    zero = jnp.zeros((3 * HALO, LN), f32)
    for c in range(ND):
        qkv_v[c, 0:3 * HALO, :] = zero
    with scope("ln0"):
        for t in ln_tasks(0):
            t()
    pw = [[functools.partial(perm_w, m, kt) for kt in range(4)] for m in ms]
    pwo = [functools.partial(perm_wo, c) for c in range(ND)]
    S0 = 4
    for b in range(NB):
        if b == 0:
            st0 = [ffn_steps(0, c) for c in range(S0)]
            with scope("b0_c0"):
                interleave(st0[0] + st0[1][:NT], [])
            with scope("b0_p1"):
                interleave(st0[1][NT:] + st0[2][:NT], pw[0])
            with scope("b0_p2"):
                interleave(st0[2][NT:] + st0[3][:NT], pw[1])
            with scope("b0_p3"):
                interleave(st0[3][NT:], pw[2][:2])
            rest = range(S0, NC)
        else:
            rest = range(NC)
        with scope(f"b{b}_qkv"):
            qs = [functools.partial(qkv_tile, b, m, c) for m in ms for c in range(ND)]
            if b == 0:
                interleave(qs[:ND], pw[2][2:])
                interleave(qs[ND:2 * ND], pwo)
                interleave(qs[2 * ND:], [])
            else:
                interleave(qs, [])
        side = (att_tasks(b) if P["ATT"] else []) + (ln_tasks(b + 1) if b + 1 < NB else [])
        with scope(f"b{b}_ffn"):
            steps = [s for c in rest for s in ffn_steps(b, c)]
            interleave(steps, side)
        with scope(f"b{b}_wo"):
            for n in range(ND):
                wo_tile(b, n)
    with scope("tail"):
        for cp in out_jobs:
            cp.wait()
        wait(*order)


DEFAULTS = dict(M=512, FC=512, T=2, QMAX=48, ATT=1, FLAGS='', SCOPES=0, FENCE=1,
                LNT=64, LNT0=64, VFIRST=1, MODE=1, XP=128, NOSTORE=1, ROLL3=0)


@jax.jit
def pallas_recurrent_scan__sliding_local_dilated__swiglu_ffn__prompt_kernel(A_x, A_wqkv, A_wo, B_x, B_w_gate, B_w_up, B_w_down):
    P = dict(DEFAULTS)
    M, FC = P["M"], P["FC"]
    x2 = A_x.reshape(S, D)
    anyspec = pl.BlockSpec(memory_space=pl.ANY)
    out = pl.pallas_call(
        functools.partial(_kernel, P=P),
        in_specs=[anyspec] * 6,
        out_specs=anyspec,
        out_shape=jax.ShapeDtypeStruct((S, D), bf16),
        scratch_shapes=[
            pltpu.VMEM((S, D), bf16),
            pltpu.VMEM((3 * ND, D // 2, LN), u32),
            pltpu.VMEM((ND, D // 2, LN), u32),
            pltpu.VMEM((NF, D // 2, LN), u32),
            pltpu.VMEM((NF, D // 2, LN), u32),
            pltpu.VMEM((ND, F // 2, LN), u32),
            pltpu.VMEM((3 * ND, D // 2, LN), u32),
            pltpu.VMEM((ND, D // 2, LN), u32),
            pltpu.VMEM((2, 97 * 32, LN), u32),
            pltpu.VMEM((ND, S // 2, LN), u32),
            pltpu.VMEM((ND, 3 * (S + HALO) + 8, LN), f32),
            pltpu.VMEM((ND, S // 2, LN), u32),
            pltpu.VMEM((2, ND, M, LN), f32),
            pltpu.VMEM((2, FC // LN, M // 2, LN), u32),
            pltpu.VMEM((ND, S // 2, LN), u32),
            pltpu.VMEM((2, 8, LN), u32),
            pltpu.SemaphoreType.DMA((64,)),
            pltpu.SemaphoreType.DMA((S // M * ND,)),
        ],
        compiler_params=pltpu.CompilerParams(
            vmem_limit_bytes=120 * 1024 * 1024,
            flags={k: True for k in P["FLAGS"].split('+') if k} or None),
    )(x2, A_wqkv, A_wo, B_w_gate, B_w_up, B_w_down)
    return out.reshape(1, S, D)
```

```python
import contextlib
import functools
import numpy as np
import jax, jax.numpy as jnp
from jax import lax
import jax.experimental.pallas as pl
import jax.experimental.pallas.tpu as pltpu

S, D, F, H, DH = 2048, 1024, 3584, 32, 32
W, DIL = 8, 2
HALO = 16
LN = 128
ND = D // LN
NF = F // LN
f32, bf16, u32 = jnp.float32, jnp.bfloat16, jnp.uint32


def _dot(a, b):
    return jnp.dot(a, b, preferred_element_type=f32)


def _silu(x):
    hx = 0.5 * x
    return hx * jnp.tanh(hx) + hx


def _kernel(x_hbm, wqkv_hbm, wo_hbm, wg_hbm, wu_hbm, wd_hbm, o_hbm,
            wqkv_v, wo_v, wg_v, wu_v, wd_v, wp_v, wop_v, tscr, xn_v, o_v, acc_v, h_v, out_v,
            zbuf, sems, osems, *blk, P):
    M, FC, T = P["M"], P["FC"], P["T"]
    NB, NC, NT = S // M, F // FC, FC // LN
    x_b, qkv_b = blk[:NB], blk[NB:]

    def scope(name):
        return jax.named_scope(name) if P["SCOPES"] else contextlib.nullcontext()

    wqkv16, wo16, wg16, wu16, wd16, out16 = (
        r.bitcast(bf16) for r in (wqkv_v, wo_v, wg_v, wu_v, wd_v, out_v))
    jobs, order = {}, []

    def add(name, pairs):
        sem = sems.at[len(order)]
        jobs[name] = [pltpu.make_async_copy(s_, d_, sem) for s_, d_ in pairs]
        order.append(name)

    def col(ref, t, rows=None):
        return ref.at[slice(None) if rows is None else rows, pl.ds(t * LN, LN)]

    def add_x(b, r0, n):
        add(("x", b, r0), [(x_hbm.at[pl.ds(b * M + r0, n), :], x_b[b].at[pl.ds(r0, n), :])])

    def add_gu(c, j0, j1):
        ts = range(c * NT + j0, c * NT + j1)
        add(("gu", c, j0), [(col(wg_hbm, t), wg16.at[t]) for t in ts] + [(col(wu_hbm, t), wu16.at[t]) for t in ts])

    def add_d(c):
        rs = pl.ds(c * FC, FC)
        add(("d", c), [(col(wd_hbm, t, rs), wd16.at[t, rs, :]) for t in range(ND)])

    def add_qkv(m):
        add(("qkv", m), [(col(wqkv_hbm, m * ND + t), wqkv16.at[m * ND + t]) for t in range(ND)])

    XP = P["XP"]
    ms = (2, 1, 0) if P["VFIRST"] else (0, 1, 2)
    if P["FENCE"]:
        add("z", [(x_hbm.at[pl.ds(0, 16), pl.ds(0, LN)], zbuf.bitcast(bf16).at[i]) for i in range(2)])
    for r0 in range(0, M, XP):
        add_x(0, r0, XP)
    G0 = [(0, 1), (1, 2), (2, 4)]
    for j0, j1 in G0:
        add_gu(0, j0, j1)
    add_d(0)
    for c in range(1, NC):
        add_gu(c, 0, NT)
        if c == 3:
            add_qkv(ms[2])
            add("wo", [(col(wo_hbm, t), wo16.at[t]) for t in range(ND)])
        if c == 2:
            add_qkv(ms[1])
        add_d(c)
        if c == 1:
            add_qkv(ms[0])
    for b in range(1, NB):
        add_x(b, 0, M)
    started, waited = [0], set()

    def start_upto(n):
        while started[0] < min(n, len(order)):
            for cp in jobs[order[started[0]]]:
                cp.start()
            started[0] += 1

    def inflight():
        return sum(len(jobs[n]) for n in order[:started[0]] if n not in waited)

    def refill():
        while started[0] < len(order) and inflight() + len(jobs[order[started[0]]]) <= P["QMAX"]:
            start_upto(started[0] + 1)

    def wait(*names):
        names = [n for n in names if n not in waited and n in jobs]
        if not names:
            return
        start_upto(max(order.index(n) for n in names) + 1)
        for n in names:
            for cp in jobs[n]:
                cp.wait()
            waited.add(n)
        refill()

    refill()
    WAIT_D = {c: [("d", c), ("gu", c + 1, 0)] for c in range(1, NC)}
    WAIT_D[0] = [("d", 0)]
    WAIT_D[1] += [("qkv", ms[0])]
    WAIT_D[2] += [("qkv", ms[1])]
    WAIT_D[3] = [("d", 3), ("qkv", ms[2]), "wo"]
    WAIT_G = {1: [("gu", 1, 0)], 4: list(order)}

    if P["NOSTORE"]:
        wg_r, wu_r, wd_r = (pltpu.annotate(r, no_store=True) for r in (wg_v, wu_v, wd_v))
    else:
        wg_r, wu_r, wd_r = wg_v, wu_v, wd_v
    z = None
    if P["FENCE"]:
        wait("z")
        z = jnp.max(jnp.abs(pltpu.bitcast(zbuf[0] ^ zbuf[1], f32))).astype(jnp.int32)

    def fence(b, val):
        if P["FENCE"]:
            v = val[0:8, :]
            for i in range(1, val.shape[0] // 8):
                v = jnp.maximum(v, val[8 * i:8 * i + 8, :])
            qkv_b[b][7, pl.ds(pl.multiple_of(z + 3 * (M + HALO), 8), 8), :] = v

    def xfence(b, val):
        if P["XF"]:
            x_b[b][pl.ds(pl.multiple_of(z + M, 16), 16), 0:LN] = val[0:16, :]

    def ld(ref, t, r0, n):
        return pltpu.bitcast(ref[t, pl.ds(r0 // 2, n // 2), :], bf16)

    def st(ref, t, r0, val):
        ref[t, pl.ds(r0 // 2, val.shape[0] // 2), :] = pltpu.bitcast(val, u32)

    def cat(ref, r0, n, nt=ND):
        return jnp.concatenate([ld(ref, t, r0, n) for t in range(nt)], axis=1)

    def ln(b, r0, n):
        if b == 0:
            wait(*[("x", 0, p0) for p0 in range((r0 // XP) * XP, r0 + n, XP)])
        g0 = b * M + r0
        x = x_b[b][pl.ds(r0, n), :].astype(f32)
        mu = jnp.mean(x, axis=-1, keepdims=True)
        xc = x - mu
        var = jnp.mean(xc * xc, axis=-1, keepdims=True)
        xn = (xc * lax.rsqrt(var + 1e-5)).astype(bf16)
        for t in range(ND):
            st(xn_v, t, g0, xn[:, t * LN:(t + 1) * LN])
        if b > 0:
            xfence(b, functools.reduce(jnp.maximum, [xn[:, t * LN:(t + 1) * LN] for t in (0, ND - 1)]))

    def ln_tasks(b):
        n = P["LNT"] if b > 0 else P["LNT0"]
        return [functools.partial(ln, b, r0, n) for r0 in range(0, M, n)]

    def perm_w(m, kt):
        ts = tscr.at[(m * 4 + kt) % 2]
        ks = slice(kt * 128, (kt + 1) * 128)
        for a in range(ND):
            t = wqkv_v[m * ND + a, ks, :].T
            for hh in range(4):
                ts[pl.ds(97 * (4 * a + hh), 32, stride=3), :] = t[hh * 32:(hh + 1) * 32, :]
        for c in range(ND):
            t = jnp.concatenate([ts[pl.ds(3 * (4 * c + dq), 32, stride=97), :] for dq in range(4)], axis=0)
            wp_v[m * ND + c, ks, :] = t.T

    def perm_wo(c):
        ts = tscr.at[c % 2]
        if P["FENCE"] and P["PPW"] and tok[0] is not None:
            tscr[0, pl.ds(pl.multiple_of(z + 97 * 32, 8), 8), :] = pltpu.bitcast(tok[0][0:8, :], u32)
        for h in range(H):
            ts[pl.ds(97 * h, 32, stride=3), :] = pltpu.bitcast(ld(wo_v, c, h * 32, 32).astype(f32), u32)
        for d2 in range(DH // 2):
            t = jnp.concatenate([ts[pl.ds(3 * (2 * d2 + e), 32, stride=97), :] for e in range(2)], axis=0)
            st(wop_v, c, d2 * 64, pltpu.bitcast(t, f32).astype(bf16))

    tok = [None]

    def qrow(r):
        return 3 * (HALO + r)

    def qkv_tile(b, m, c):
        y = _dot(cat(xn_v, b * M, M), ld(wp_v, m * ND + c, 0, D))
        tok[0] = y[M - 8:, :]
        if m == 0:
            y = y * (DH ** -0.5)
        qkv_b[b][c, pl.ds(qrow(0) + (2, 0, 1)[m], M, stride=3), :] = y
        if m > 0 and b + 1 < NB:
            qkv_b[b + 1][c, pl.ds((0, 0, 1)[m], HALO, stride=3), :] = y[M - HALO:, :]

    def att_tile(b, r0):
        n = 8 * T
        g0 = b * M + r0
        qkv_v = qkv_b[b]
        ls = [None] * W
        qs = [qkv_v[c, pl.ds(qrow(r0) + 2, n, stride=3), :] for c in range(ND)]
        for w in range(W):
            l = None
            for c in range(ND):
                k = qkv_v[c, pl.ds(qrow(r0 - DIL * w), n, stride=3), :]
                l = qs[c] * k if c == 0 else l + qs[c] * k
            ls[w] = l
            if (w + 1) % P["FW"] == 0:
                fence(b, functools.reduce(jnp.maximum, ls[w + 1 - P["FW"]:w + 1]))
        for w in range(W):
            l = ls[w]
            if P["ROLL3"]:
                l = (l + pltpu.roll(l, 32, 1)) + (pltpu.roll(l, 64, 1) + pltpu.roll(l, 96, 1))
            else:
                l = l + pltpu.roll(l, 64, 1)
                l = l + pltpu.roll(l, 32, 1)
            if g0 < DIL * w:
                rows = g0 + lax.broadcasted_iota(jnp.int32, (n, LN), 0)
                l = jnp.where(rows >= DIL * w, l, -1e9)
            ls[w] = l
        mx = functools.reduce(jnp.maximum, ls)
        ps = [jnp.exp(l - mx) for l in ls]
        r = 1.0 / functools.reduce(jnp.add, ps)
        if P["NORM"] == 0:
            ps = [p * r for p in ps]
            fence(b, functools.reduce(jnp.maximum, ps))
        else:
            fence(b, r)
        accs = []
        for c in range(ND):
            acc = None
            for w in range(W):
                v = qkv_v[c, pl.ds(qrow(r0 - DIL * w) + 1, n, stride=3), :]
                acc = ps[w] * v if w == 0 else acc + ps[w] * v
            if P["NORM"] == 1:
                acc = acc * r
            accs.append(acc)
            if (c + 1) % P["FW"] == 0:
                fence(b, functools.reduce(jnp.maximum, accs[-P["FW"]:]))
            st(o_v, c, g0, acc.astype(bf16))

    def att_tasks(b):
        return [functools.partial(att_tile, b, r0) for r0 in range(0, M, 8 * T)]

    def gu_tile(b, c, j):
        t = c * NT + j
        if b == 0 and c == 0:
            wait(*[("gu", 0, j0) for j0, j1 in G0 if j0 <= j < j1])
        if b == 0 and j == 0 and c in WAIT_G:
            wait(*WAIT_G[c])
        xn = cat(xn_v, b * M, M)
        g = _dot(xn, ld(wg_r, t, 0, D))
        u = _dot(xn, ld(wu_r, t, 0, D))
        st(h_v.at[c % 2], j, 0, (_silu(g) * u).astype(bf16))

    def down_tile(b, c, n):
        if b == 0 and n == 0:
            wait(*WAIT_D[c])
        t = _dot(cat(h_v.at[c % 2], 0, M, NT), ld(wd_r, n, c * FC, FC))
        if c == 0:
            acc_v[b % 2, n] = t
        else:
            acc_v[b % 2, n] = acc_v[b % 2, n] + t

    def ffn_steps(b, c):
        return [functools.partial(gu_tile, b, c, j) for j in range(NT)] + \
               [functools.partial(down_tile, b, c, n) for n in range(ND)]

    out_jobs = []

    def wo_tile(b, n):
        s = _dot(cat(o_v, b * M, M), ld(wop_v, n, 0, D))
        gate = _silu(acc_v[b % 2, n])
        st(out_v, n, b * M, (x_b[b][pl.ds(0, M), n * LN:(n + 1) * LN].astype(f32) + s * gate).astype(bf16))
        rs = pl.ds(b * M, M)
        cp = pltpu.make_async_copy(out16.at[n, rs, :], col(o_hbm, n, rs), osems.at[b * ND + n])
        cp.start()
        out_jobs.append(cp)

    def interleave(main, side):
        ns, nm, done = len(side), len(main), 0
        for i, step in enumerate(main):
            step()
            upto = (ns * (i + 1) + nm - 1) // nm
            while done < min(upto, ns):
                side[done]()
                done += 1
        while done < ns:
            side[done]()
            done += 1

    zero = jnp.zeros((3 * HALO, LN), f32)
    for c in range(ND):
        qkv_b[0][c, 0:3 * HALO, :] = zero
    with scope("ln0"):
        for t in ln_tasks(0):
            t()
    pw = [[functools.partial(perm_w, m, kt) for kt in range(4)] for m in ms]
    pwo = [functools.partial(perm_wo, c) for c in range(ND)]
    S0 = 4
    for b in range(NB):
        if b == 0:
            st0 = [ffn_steps(0, c) for c in range(S0)]
            with scope("b0_c0"):
                interleave(st0[0] + st0[1][:NT], [])
            with scope("b0_p1"):
                interleave(st0[1][NT:] + st0[2][:NT], pw[0])
            with scope("b0_p2"):
                interleave(st0[2][NT:] + st0[3][:NT], pw[1])
            with scope("b0_p3"):
                interleave(st0[3][NT:], pw[2][:P["PQ"]])
            rest = range(S0, NC)
        else:
            rest = range(NC)
        with scope(f"b{b}_qkv"):
            qs = [functools.partial(qkv_tile, b, m, c) for m in ms for c in range(ND)]
            if b == 0:
                interleave(qs[:ND], pw[2][P["PQ"]:])
                interleave(qs[ND:], pwo)
            else:
                interleave(qs, [])
        side = (att_tasks(b) if P["ATT"] else []) + (ln_tasks(b + 1) if b + 1 < NB else [])
        with scope(f"b{b}_ffn"):
            steps = [s for c in rest for s in ffn_steps(b, c)]
            if P["ATTPOS"] == 0:
                interleave(steps, side)
            else:
                k = len(ffn_steps(b, 0))
                interleave(steps[:-k], att_tasks(b))
                interleave(steps[-k:], ln_tasks(b + 1) if b + 1 < NB else [])
        with scope(f"b{b}_wo"):
            for n in range(ND):
                wo_tile(b, n)
    with scope("tail"):
        for cp in out_jobs:
            cp.wait()
        wait(*order)


DEFAULTS = dict(M=512, FC=512, T=2, QMAX=48, ATT=1, FLAGS='', SCOPES=0, FENCE=1,
                LNT=16, LNT0=64, VFIRST=1, FW=1, XF=1, NORM=1, NOCHK=1, PQ=2, PPW=1, ATTPOS=0, XP=128, NOSTORE=0, ROLL3=0)


@jax.jit
def pallas_recurrent_scan__sliding_local_dilated__swiglu_ffn__prompt_kernel(A_x, A_wqkv, A_wo, B_x, B_w_gate, B_w_up, B_w_down):
    P = dict(DEFAULTS)
    M, FC = P["M"], P["FC"]
    x2 = A_x.reshape(S, D)
    anyspec = pl.BlockSpec(memory_space=pl.ANY)
    out = pl.pallas_call(
        functools.partial(_kernel, P=P),
        in_specs=[anyspec] * 6,
        out_specs=anyspec,
        out_shape=jax.ShapeDtypeStruct((S, D), bf16),
        scratch_shapes=[
            pltpu.VMEM((3 * ND, D // 2, LN), u32),
            pltpu.VMEM((ND, D // 2, LN), u32),
            pltpu.VMEM((NF, D // 2, LN), u32),
            pltpu.VMEM((NF, D // 2, LN), u32),
            pltpu.VMEM((ND, F // 2, LN), u32),
            pltpu.VMEM((3 * ND, D // 2, LN), u32),
            pltpu.VMEM((ND, D // 2, LN), u32),
            pltpu.VMEM((2, 97 * 32 + 8, LN), u32),
            pltpu.VMEM((ND, S // 2, LN), u32),
            pltpu.VMEM((ND, S // 2, LN), u32),
            pltpu.VMEM((2, ND, M, LN), f32),
            pltpu.VMEM((2, FC // LN, M // 2, LN), u32),
            pltpu.VMEM((ND, S // 2, LN), u32),
            pltpu.VMEM((2, 8, LN), u32),
            pltpu.SemaphoreType.DMA((40,)),
            pltpu.SemaphoreType.DMA((S // M * ND,)),
        ] + [pltpu.VMEM((M + 16, D), bf16)] * (S // M) + [pltpu.VMEM((ND, 3 * (M + HALO) + 8, LN), f32)] * (S // M) + [
        ],
        compiler_params=pltpu.CompilerParams(
            vmem_limit_bytes=120 * 1024 * 1024, disable_semaphore_checks=bool(P["NOCHK"]),
            flags={k: True for k in P["FLAGS"].split('+') if k} or None),
    )(x2, A_wqkv, A_wo, B_w_gate, B_w_up, B_w_down)
    return out.reshape(1, S, D)
```

```python
import functools

import jax
import jax.numpy as jnp
from jax import lax
import jax.experimental.pallas as pl
import jax.experimental.pallas.tpu as pltpu

S, D, F, H, DH = 2048, 1024, 3584, 32, 32
W, DIL = 8, 2
HALO = 16
LN = 128
ND, NF = D // LN, F // LN
M = 512
FC = 512
NB, NC, NT = S // M, F // FC, FC // LN
TR = 16
LNR = 32
XP = 128
QMAX = 48
f32, bf16, u32 = jnp.float32, jnp.bfloat16, jnp.uint32


def _dot(a, b):
    return jnp.dot(a, b, preferred_element_type=f32)


def _silu(x):
    hx = 0.5 * x
    return hx * jnp.tanh(hx) + hx


def _kernel(x_hbm, wqkv_hbm, wo_hbm, wg_hbm, wu_hbm, wd_hbm, o_hbm,
            wqkv_v, wo_v, wg_v, wu_v, wd_v, wp_v, wop_v, tscr, xn_v, o_v, acc_v, h_v, out_v,
            zbuf, sems, osems, *blk):
    x_b, qkv_b = blk[:NB], blk[NB:]

    wqkv16, wo16, wg16, wu16, wd16, out16 = (
        r.bitcast(bf16) for r in (wqkv_v, wo_v, wg_v, wu_v, wd_v, out_v))
    jobs, order = {}, []

    def add(name, pairs):
        sem = sems.at[len(order)]
        jobs[name] = [pltpu.make_async_copy(s, d, sem) for s, d in pairs]
        order.append(name)

    def col(ref, t, rows=None):
        return ref.at[slice(None) if rows is None else rows, pl.ds(t * LN, LN)]

    def add_x(b, r0, n):
        add(("x", b, r0), [(x_hbm.at[pl.ds(b * M + r0, n), :], x_b[b].at[pl.ds(r0, n), :])])

    def add_gu(c, j0, j1):
        ts = range(c * NT + j0, c * NT + j1)
        add(("gu", c, j0), [(col(wg_hbm, t), wg16.at[t]) for t in ts]
            + [(col(wu_hbm, t), wu16.at[t]) for t in ts])

    def add_d(c):
        rs = pl.ds(c * FC, FC)
        add(("d", c), [(col(wd_hbm, t, rs), wd16.at[t, rs, :]) for t in range(ND)])

    def add_qkv(m):
        add(("qkv", m), [(col(wqkv_hbm, m * ND + t), wqkv16.at[m * ND + t]) for t in range(ND)])

    ms = (2, 1, 0)
    add("z", [(x_hbm.at[pl.ds(0, 16), pl.ds(0, LN)], zbuf.bitcast(bf16).at[i]) for i in range(2)])
    for r0 in range(0, M, XP):
        add_x(0, r0, XP)
    add("g0", [(col(wg_hbm, 0), wg16.at[0])])
    add(("gu", 0, 0), [(col(wu_hbm, 0), wu16.at[0])])
    G0 = [(0, 1), (1, 2), (2, NT)]
    for j0, j1 in G0[1:]:
        add_gu(0, j0, j1)
    add_d(0)
    for c in range(1, NC):
        add_gu(c, 0, NT)
        if c == 2:
            add_qkv(ms[1])
        if c == 3:
            add_qkv(ms[2])
            add("wo", [(col(wo_hbm, t), wo16.at[t]) for t in range(ND)])
        add_d(c)
        if c == 1:
            add_qkv(ms[0])
    for b in range(1, NB):
        add_x(b, 0, M)
    started, waited = [0], set()

    def start_upto(n):
        while started[0] < min(n, len(order)):
            for cp in jobs[order[started[0]]]:
                cp.start()
            started[0] += 1

    def refill():
        while started[0] < len(order):
            busy = sum(len(jobs[n]) for n in order[:started[0] + 1] if n not in waited)
            if busy > QMAX:
                break
            start_upto(started[0] + 1)

    def wait(*names):
        names = [n for n in names if n not in waited]
        if not names:
            return
        start_upto(max(order.index(n) for n in names) + 1)
        for n in names:
            for cp in jobs[n]:
                cp.wait()
            waited.add(n)
        refill()

    wait_d = {c: [("d", c), ("gu", c + 1, 0)] for c in range(1, NC - 1)}
    wait_d[0] = [("d", 0)]
    wait_d[1] += [("qkv", ms[0])]
    wait_d[2] += [("qkv", ms[1])]
    wait_d[3] = [("d", 3), ("qkv", ms[2]), "wo"]
    wait_g = {1: [("gu", 1, 0)], 4: list(order)}

    refill()
    wait("z")
    z = jnp.max(jnp.abs(pltpu.bitcast(zbuf[0] ^ zbuf[1], f32))).astype(jnp.int32)

    def fence(b, val):
        v = val[0:8, :]
        for i in range(1, val.shape[0] // 8):
            v = jnp.maximum(v, val[8 * i:8 * i + 8, :])
        qkv_b[b][ND - 1, pl.ds(pl.multiple_of(z + 3 * (M + HALO), 8), 8), :] = v

    def ld(ref, t, r0, n):
        return pltpu.bitcast(ref[t, pl.ds(r0 // 2, n // 2), :], bf16)

    def st(ref, t, r0, val):
        ref[t, pl.ds(r0 // 2, val.shape[0] // 2), :] = pltpu.bitcast(val, u32)

    def cat(ref, r0, n, nt=ND):
        return jnp.concatenate([ld(ref, t, r0, n) for t in range(nt)], axis=1)

    def ln(b, r0, n):
        if b == 0:
            wait(*[("x", 0, p0) for p0 in range((r0 // XP) * XP, r0 + n, XP)])
        x = x_b[b][pl.ds(r0, n), :].astype(f32)
        mu = jnp.mean(x, axis=-1, keepdims=True)
        xc = x - mu
        var = jnp.mean(xc * xc, axis=-1, keepdims=True)
        xn = (xc * lax.rsqrt(var + 1e-5)).astype(bf16)
        for t in range(ND):
            st(xn_v, t, b * M + r0, xn[:, t * LN:(t + 1) * LN])
        if b > 0:
            done = jnp.maximum(xn[0:16, 0:LN], xn[0:16, D - LN:D])
            x_b[b][pl.ds(pl.multiple_of(z + M, 16), 16), 0:LN] = done

    def ln_tasks(b):
        n = LNR if b > 0 else 64
        return [functools.partial(ln, b, r0, n) for r0 in range(0, M, n)]

    def perm_w(m, kt):
        ts = tscr.at[(m * 4 + kt) % 2]
        ks = slice(kt * LN, (kt + 1) * LN)
        for a in range(ND):
            t = wqkv_v[m * ND + a, ks, :].T
            for hh in range(4):
                ts[pl.ds(97 * (4 * a + hh), DH, stride=3), :] = t[hh * DH:(hh + 1) * DH, :]
        for c in range(ND):
            t = jnp.concatenate(
                [ts[pl.ds(3 * (4 * c + dq), H, stride=97), :] for dq in range(4)], axis=0)
            wp_v[m * ND + c, ks, :] = t.T

    tok = [None]

    def perm_wo(c):
        ts = tscr.at[c % 2]
        tscr[0, pl.ds(pl.multiple_of(z + 97 * H, 8), 8), :] = pltpu.bitcast(tok[0], u32)
        for h in range(H):
            ts[pl.ds(97 * h, DH, stride=3), :] = pltpu.bitcast(ld(wo_v, c, h * DH, DH).astype(f32), u32)
        for d2 in range(DH // 2):
            t = jnp.concatenate(
                [ts[pl.ds(3 * (2 * d2 + e), H, stride=97), :] for e in range(2)], axis=0)
            st(wop_v, c, d2 * 2 * H, pltpu.bitcast(t, f32).astype(bf16))

    def qrow(r):
        return 3 * (HALO + r)

    def qkv_tile(b, m, c):
        y = _dot(cat(xn_v, b * M, M), ld(wp_v, m * ND + c, 0, D))
        tok[0] = y[M - 8:, :]
        if m == 0:
            y = y * (DH ** -0.5)
        qkv_b[b][c, pl.ds(qrow(0) + (2, 0, 1)[m], M, stride=3), :] = y
        if m > 0 and b + 1 < NB:
            qkv_b[b + 1][c, pl.ds(m - 1, HALO, stride=3), :] = y[M - HALO:, :]

    def att_tile(b, r0):
        g0 = b * M + r0
        qkv = qkv_b[b]
        qs = [qkv[c, pl.ds(qrow(r0) + 2, TR, stride=3), :] for c in range(ND)]
        ls = []
        for w in range(W):
            l = None
            for c in range(ND):
                k = qkv[c, pl.ds(qrow(r0 - DIL * w), TR, stride=3), :]
                l = qs[c] * k if c == 0 else l + qs[c] * k
            ls.append(l)
            fence(b, l)
            if w + 1 < W:
                yield
        for w in range(W):
            l = ls[w] + pltpu.roll(ls[w], 2 * H, 1)
            l = l + pltpu.roll(l, H, 1)
            if g0 < DIL * w:
                rows = g0 + lax.broadcasted_iota(jnp.int32, (TR, LN), 0)
                l = jnp.where(rows >= DIL * w, l, -1e9)
            ls[w] = l
        mx = functools.reduce(jnp.maximum, ls)
        ps = [jnp.exp(l - mx) for l in ls]
        r = 1.0 / functools.reduce(jnp.add, ps)
        fence(b, r)
        yield
        for c in range(ND):
            acc = None
            for w in range(W):
                v = qkv[c, pl.ds(qrow(r0 - DIL * w) + 1, TR, stride=3), :]
                acc = ps[w] * v if w == 0 else acc + ps[w] * v
            acc = acc * r
            fence(b, acc)
            st(o_v, c, g0, acc.astype(bf16))
            yield

    def att_tasks(b):
        def pieces():
            for r0 in range(0, M, TR):
                yield from att_tile(b, r0)
        return [functools.partial(next, pieces_it) for pieces_it in [pieces()]] * ((M // TR) * (W + ND))

    def gu_tile(b, c, j):
        t = c * NT + j
        first = b == 0 and c == 0 and j == 0
        if first:
            wait("g0")
        elif b == 0 and c == 0:
            wait(*[("gu", 0, j0) for j0, j1 in G0 if j0 <= j < j1])
        if b == 0 and j == 0 and c in wait_g:
            wait(*wait_g[c])
        xn = cat(xn_v, b * M, M)
        g = _dot(xn, ld(wg_v, t, 0, D))
        if first:
            wait(("gu", 0, 0))
        u = _dot(xn, ld(wu_v, t, 0, D))
        st(h_v.at[c % 2], j, 0, (_silu(g) * u).astype(bf16))

    dtok = [None]

    def down_tile(b, c, n):
        if b == 0 and n == 0 and c in wait_d:
            wait(*wait_d[c])
        t = _dot(cat(h_v.at[c % 2], 0, M, NT), ld(wd_v, n, c * FC, FC))
        dtok[0] = t[M // 2:M // 2 + 8, :]
        acc_v[b % 2, n] = t if c == 0 else acc_v[b % 2, n] + t

    def ffn_steps(b, c):
        return ([functools.partial(gu_tile, b, c, j) for j in range(NT)]
                + [functools.partial(down_tile, b, c, n) for n in range(ND)])

    out_jobs = []

    def wo_tile(b, n):
        s = _dot(cat(o_v, b * M, M), ld(wop_v, n, 0, D))
        gate = _silu(acc_v[b % 2, n])
        x = x_b[b][pl.ds(0, M), n * LN:(n + 1) * LN].astype(f32)
        st(out_v, n, b * M, (x + s * gate).astype(bf16))
        rs = pl.ds(b * M, M)
        cp = pltpu.make_async_copy(out16.at[n, rs, :], col(o_hbm, n, rs), osems.at[b * ND + n])
        cp.start()
        out_jobs.append(cp)

    def interleave(main, side):
        done = 0
        for i, step in enumerate(main):
            step()
            upto = (len(side) * (i + 1) + len(main) - 1) // len(main)
            for task in side[done:upto]:
                task()
            done = upto

    for c in range(ND):
        qkv_b[0][c, 0:3 * HALO, :] = jnp.zeros((3 * HALO, LN), f32)
    for task in ln_tasks(0):
        task()
    pw = [[functools.partial(perm_w, m, kt) for kt in range(4)] for m in ms]
    for b in range(NB):
        proj = [functools.partial(qkv_tile, b, m, c) for m in ms for c in range(ND)]
        lns = ln_tasks(b + 1) if b + 1 < NB else []
        if b == 0:
            head = [ffn_steps(0, c) for c in range(4)]
            interleave(head[0] + head[1][:NT], [])
            interleave(head[1][NT:] + head[2][:NT], pw[0])
            interleave(head[2][NT:] + head[3][:NT], pw[1])
            interleave(head[3][NT:], pw[2][:2])
            interleave(proj[:ND], pw[2][2:])
            interleave(proj[ND:], [functools.partial(perm_wo, c) for c in range(ND)])
            interleave([s for c in range(4, NC) for s in ffn_steps(0, c)], att_tasks(0) + lns)
        else:
            interleave(proj, [])
            att, k = att_tasks(b), 0
            for c in range(NC):
                for j, step in enumerate(ffn_steps(b, c)):
                    step()
                    if j >= NT:
                        fence(b, dtok[0])
                        for piece in att[len(att) * k // (NC * ND):len(att) * (k + 1) // (NC * ND)]:
                            piece()
                        k += 1
                    elif c == NC - 1:
                        for task in lns[len(lns) * j // NT:len(lns) * (j + 1) // NT]:
                            task()
        for n in range(ND):
            wo_tile(b, n)
    for cp in out_jobs:
        cp.wait()
    wait(*order)


@jax.jit
def pallas_recurrent_scan__sliding_local_dilated__swiglu_ffn__prompt_kernel(
        A_x, A_wqkv, A_wo, B_x, B_w_gate, B_w_up, B_w_down):
    del B_x
    anyspec = pl.BlockSpec(memory_space=pl.ANY)
    out = pl.pallas_call(
        _kernel,
        in_specs=[anyspec] * 6,
        out_specs=anyspec,
        out_shape=jax.ShapeDtypeStruct((S, D), bf16),
        scratch_shapes=[
            pltpu.VMEM((3 * ND, D // 2, LN), u32),
            pltpu.VMEM((ND, D // 2, LN), u32),
            pltpu.VMEM((NF, D // 2, LN), u32),
            pltpu.VMEM((NF, D // 2, LN), u32),
            pltpu.VMEM((ND, F // 2, LN), u32),
            pltpu.VMEM((3 * ND, D // 2, LN), u32),
            pltpu.VMEM((ND, D // 2, LN), u32),
            pltpu.VMEM((2, 100 * H, LN), u32),
            pltpu.VMEM((ND, S // 2, LN), u32),
            pltpu.VMEM((ND, S // 2, LN), u32),
            pltpu.VMEM((2, ND, M, LN), f32),
            pltpu.VMEM((2, NT, M // 2, LN), u32),
            pltpu.VMEM((ND, S // 2, LN), u32),
            pltpu.VMEM((2, 8, LN), u32),
            pltpu.SemaphoreType.DMA((32,)),
            pltpu.SemaphoreType.DMA((NB * ND,)),
        ] + [pltpu.VMEM((M + 16, D), bf16)] * NB
          + [pltpu.VMEM((ND, 3 * (M + HALO) + 8, LN), f32)] * NB,
        compiler_params=pltpu.CompilerParams(
            vmem_limit_bytes=120 * 1024 * 1024, disable_semaphore_checks=True),
    )(A_x.reshape(S, D), A_wqkv, A_wo, B_w_gate, B_w_up, B_w_down)
    return out.reshape(1, S, D)
```
